```python
import os as _os
_os.environ.setdefault("JAX_PLATFORMS", "cpu")
import jax
import jax.numpy as jnp

def _softmax(x, axis=-1):
    return jax.nn.softmax(x, axis=axis)
def _gelu(x):
    return jax.nn.gelu(x, approximate=True)
def _silu(x):
    return jax.nn.silu(x)
def _sigmoid(x):
    return jax.nn.sigmoid(x)
def _layernorm(x, axis=-1, eps=1e-5):
    m = jnp.mean(x, axis=axis, keepdims=True)
    v = jnp.var(x, axis=axis, keepdims=True)
    return (x - m) / jnp.sqrt(v + eps)
def _scatter_add(tgt, idx, src, axis=0):
    return tgt.at[idx].add(src)
def _segment_sum(src, seg, n):
    return jax.ops.segment_sum(src, seg, n)
class _Rng:
    def __init__(self, key):
        self._k = key
    def _next(self):
        self._k, sub = jax.random.split(self._k)
        return sub
    def normal(self, shape):
        return jax.random.normal(self._next(), shape, dtype=jnp.bfloat16)
    def randint(self, lo, hi, shape):
        return jax.random.randint(self._next(), shape, lo, hi, dtype=jnp.int32)
    def uniform(self, shape, lo=0.0, hi=1.0):
        return jax.random.uniform(self._next(), shape, jnp.bfloat16, lo, hi)
    def permutation(self, n):
        return jax.random.permutation(self._next(), n)


kernel_name = 'standalone__instancenorm__sampling'

def setup_inputs():
    _rng = _Rng(jax.random.key(int.from_bytes(__import__("os").urandom(4), "little")))
    _w = (lambda a: (lambda t: t.astype(jnp.bfloat16) if jnp.issubdtype(t.dtype, jnp.floating) else t)(jnp.asarray(a)))
    B, C, H, W = 16, 640, 16, 32
    return {
        "x": _w((lambda *s: _rng.normal(s) * 0.05)(B, C, H, W)),
        "g": _w((lambda *s: _rng.normal(s) * 0.05)(C) + 1.0),
        "b": _w((lambda *s: _rng.normal(s) * 0.05)(C)),
    }

def reference(x, g, b):
    mu = x.mean(axis=(-2, -1), keepdims=True)
    var = ((x - mu) * (x - mu)).mean(axis=(-2, -1), keepdims=True)
    xhat = (x - mu) / jnp.sqrt(var + 1e-5)
    return xhat * g.reshape(1, -1, 1, 1) + b.reshape(1, -1, 1, 1)
```

```python
import jax
import jax.numpy as jnp
from jax import lax
import jax.experimental.pallas as pl
import jax.experimental.pallas.tpu as pltpu

_EPS = 1e-5
_LANES = 128
_NUM_READS = 4


def _normalize_batch(buf, gamma, beta, b, *, hw, c):
    inv_hw = 1.0 / hw
    for c0 in range(0, c, 2 * _LANES):
        width = min(2 * _LANES, c - c0)
        cols = pl.ds(c0, width)
        tiles = range(c0 // _LANES, (c0 + width) // _LANES)
        g = jnp.concatenate([gamma[j:j + 1, :] for j in tiles], axis=1)
        bias = jnp.concatenate([beta[j:j + 1, :] for j in tiles], axis=1)

        x = buf[b, :, cols].astype(jnp.float32)
        mu = jnp.sum(x, axis=0, keepdims=True) * inv_hw
        d = x - mu
        var = jnp.sum(d * d, axis=0, keepdims=True) * inv_hw
        scale = lax.rsqrt(var + _EPS) * g
        buf[b, :, cols] = (d * scale + bias).astype(buf.dtype)


def _instancenorm_kernel(x_hbm, g_hbm, b_hbm, o_hbm, buf, g_vmem, b_vmem, read_sem, write_sem,
                         gb_sem):
    nb, hw, c = x_hbm.shape
    per_read = nb // _NUM_READS
    last0 = nb - per_read

    def read(i):
        rows = pl.ds(i * per_read, per_read)
        return pltpu.make_async_copy(x_hbm.at[rows], buf.at[rows], read_sem.at[i])

    def write(start, size, slot):
        rows = pl.ds(start, size)
        return pltpu.make_async_copy(buf.at[rows], o_hbm.at[rows], write_sem.at[slot])

    write_head = write(0, last0, 0)
    write_tail = write(last0, per_read, 1)

    load_g = pltpu.make_async_copy(g_hbm, g_vmem, gb_sem.at[0])
    load_b = pltpu.make_async_copy(b_hbm, b_vmem, gb_sem.at[1])
    read(0).start()
    load_g.start()
    load_b.start()

    def start_read(i, carry):
        read(i).start()
        return carry

    lax.fori_loop(1, _NUM_READS, start_read, 0)
    load_g.wait()
    load_b.wait()
    gamma = g_vmem[...].astype(jnp.float32)
    beta = b_vmem[...].astype(jnp.float32)

    def body(b, carry):
        @pl.when(b % per_read == 0)
        def _():
            read(b // per_read).wait()

        @pl.when(b == last0)
        def _():
            write_head.start()

        _normalize_batch(buf, gamma, beta, b, hw=hw, c=c)
        return carry

    lax.fori_loop(0, nb, body, 0)
    write_tail.start()
    write_head.wait()
    write_tail.wait()


@jax.jit
def pallas_standalone__instancenorm__sampling_kernel(
    x: jax.Array,
    g: jax.Array,
    b: jax.Array,
):
    nb, c, h, w = x.shape
    hw = h * w
    assert c % _LANES == 0 and nb % _NUM_READS == 0 and hw % 16 == 0

    x_rows = jnp.transpose(x, (0, 2, 3, 1)).reshape(nb, hw, c)
    g_tiles = g.reshape(c // _LANES, _LANES)
    b_tiles = b.reshape(c // _LANES, _LANES)

    any_spec = pl.BlockSpec(memory_space=pl.ANY)
    out_rows = pl.pallas_call(
        _instancenorm_kernel,
        in_specs=[any_spec, any_spec, any_spec],
        out_specs=any_spec,
        out_shape=jax.ShapeDtypeStruct((nb, hw, c), x.dtype),
        scratch_shapes=[
            pltpu.VMEM((nb, hw, c), x.dtype),
            pltpu.VMEM(g_tiles.shape, g.dtype),
            pltpu.VMEM(b_tiles.shape, b.dtype),
            pltpu.SemaphoreType.DMA((_NUM_READS,)),
            pltpu.SemaphoreType.DMA((2,)),
            pltpu.SemaphoreType.DMA((2,)),
        ],
        compiler_params=pltpu.CompilerParams(vmem_limit_bytes=48 * 1024 * 1024),
    )(x_rows, g_tiles, b_tiles)
    return jnp.transpose(out_rows.reshape(nb, h, w, c), (0, 3, 1, 2))
```

```python
import jax
import jax.numpy as jnp
from jax import lax
import jax.experimental.pallas as pl
import jax.experimental.pallas.tpu as pltpu

_EPS = 1e-5
_LANES = 128
_SUBLANES = 8
_WRITE_ROWS = 16
_DRAIN_ROWS = 256
_NUM_ACC = 4


def _tree_sum(vals):
    vals = list(vals)
    while len(vals) > 1:
        vals = [vals[i] + vals[i + 1] if i + 1 < len(vals) else vals[i]
                for i in range(0, len(vals), 2)]
    return vals[0]


def _normalize_batch(buf, gamma, beta, batch_ids, *, hw, c):
    rt = _SUBLANES
    n_tiles = hw // rt
    inv_hw = 1.0 / hw
    mean_view, var_view, out_view = (buf.at[i] for i in batch_ids)

    for c0 in range(0, c, 2 * _LANES):
        width = min(2 * _LANES, c - c0)
        cols = pl.ds(c0, width)
        tiles = range(c0 // _LANES, (c0 + width) // _LANES)
        g = jnp.concatenate([gamma[j:j + 1, :] for j in tiles], axis=1)
        bias = jnp.concatenate([beta[j:j + 1, :] for j in tiles], axis=1)

        def load(view, r):
            return view[pl.ds(r * rt, rt), cols].astype(jnp.float32)

        def column_mean(term):
            acc = [None] * _NUM_ACC
            for r in range(n_tiles):
                t = term(r)
                k = r % _NUM_ACC
                acc[k] = t if acc[k] is None else acc[k] + t
            return jnp.sum(_tree_sum(acc), axis=0, keepdims=True) * inv_hw

        mu = jnp.broadcast_to(column_mean(lambda r: load(mean_view, r)), (rt, width))

        def centered_square(r):
            d = load(var_view, r) - mu
            return d * d

        var = column_mean(centered_square)
        scale = jnp.broadcast_to(lax.rsqrt(var + _EPS) * g, (rt, width))
        shift = jnp.broadcast_to(bias, (rt, width))
        for r in range(n_tiles):
            out = (load(out_view, r) - mu) * scale + shift
            out_view[pl.ds(r * rt, rt), cols] = out.astype(buf.dtype)


def _instancenorm_kernel(x_hbm, g_hbm, b_hbm, o_hbm, buf, g_vmem, b_vmem, read_sem, write_sem,
                         gb_sem):
    nb, hw, c = x_hbm.shape
    half = nb // 2
    last = nb - 1
    drain = min(_DRAIN_ROWS, hw // 2)

    def batches_read(i, b0, n):
        rows = pl.ds(b0, n)
        return pltpu.make_async_copy(x_hbm.at[rows], buf.at[rows], read_sem.at[i])

    def rows_read(i, r0, n):
        rows = pl.ds(r0, n)
        return pltpu.make_async_copy(x_hbm.at[last, rows], buf.at[last, rows], read_sem.at[i])

    reads = (
        batches_read(0, 0, half),
        batches_read(1, half, last - half),
        rows_read(2, 0, hw - drain),
        rows_read(3, hw - drain, drain),
    )

    def writes(b0, n, slot):
        batches = pl.ds(b0, n)
        return [
            pltpu.make_async_copy(buf.at[batches, pl.ds(r0, _WRITE_ROWS)],
                                  o_hbm.at[batches, pl.ds(r0, _WRITE_ROWS)],
                                  write_sem.at[slot])
            for r0 in range(0, hw, _WRITE_ROWS)
        ]

    writes_head = writes(0, half, 0)
    writes_tail = writes(half, nb - half, 1)

    load_g = pltpu.make_async_copy(g_hbm, g_vmem, gb_sem.at[0])
    load_b = pltpu.make_async_copy(b_hbm, b_vmem, gb_sem.at[1])
    reads[0].start()
    load_g.start()
    load_b.start()

    def start_read(i, carry):
        for k in range(1, len(reads)):
            @pl.when(i == k)
            def _():
                reads[k].start()
        return carry

    lax.fori_loop(1, len(reads), start_read, 0, unroll=False)
    load_g.wait()
    load_b.wait()
    gamma = g_vmem[...].astype(jnp.float32)
    beta = b_vmem[...].astype(jnp.float32)

    def body(b, carry):
        b_var, b_out = carry

        @pl.when(b == 0)
        def _():
            reads[0].wait()

        @pl.when(b == half)
        def _():
            reads[1].wait()
            reads[2].wait()
            for copy in writes_head:
                copy.start()

        @pl.when(b == last)
        def _():
            reads[3].wait()

        _normalize_batch(buf, gamma, beta, (b, b_var, b_out), hw=hw, c=c)
        return b_var + 1, b_out + 1

    lax.fori_loop(0, nb, body, (jnp.int32(0), jnp.int32(0)))
    for copy in writes_tail:
        copy.start()
    for copy in writes_head:
        copy.wait()
    for copy in writes_tail:
        copy.wait()


@jax.jit
def pallas_standalone__instancenorm__sampling_kernel(
    x: jax.Array,
    g: jax.Array,
    b: jax.Array,
):
    nb, c, h, w = x.shape
    hw = h * w
    assert c % _LANES == 0 and nb >= 4 and hw % (2 * _WRITE_ROWS) == 0

    x_rows = jnp.transpose(x, (0, 2, 3, 1)).reshape(nb, hw, c)
    g_tiles = g.reshape(c // _LANES, _LANES)
    b_tiles = b.reshape(c // _LANES, _LANES)

    any_spec = pl.BlockSpec(memory_space=pl.ANY)
    out_rows = pl.pallas_call(
        _instancenorm_kernel,
        in_specs=[any_spec, any_spec, any_spec],
        out_specs=any_spec,
        out_shape=jax.ShapeDtypeStruct((nb, hw, c), x.dtype),
        scratch_shapes=[
            pltpu.VMEM((nb, hw, c), x.dtype),
            pltpu.VMEM(g_tiles.shape, g.dtype),
            pltpu.VMEM(b_tiles.shape, b.dtype),
            pltpu.SemaphoreType.DMA((4,)),
            pltpu.SemaphoreType.DMA((2,)),
            pltpu.SemaphoreType.DMA((2,)),
        ],
        compiler_params=pltpu.CompilerParams(vmem_limit_bytes=32 * 1024 * 1024),
    )(x_rows, g_tiles, b_tiles)
    return jnp.transpose(out_rows.reshape(nb, h, w, c), (0, 3, 1, 2))
```
